```python
import os as _os
_os.environ.setdefault("JAX_PLATFORMS", "cpu")
import jax
import jax.numpy as jnp

def _softmax(x, axis=-1):
    return jax.nn.softmax(x, axis=axis)
def _gelu(x):
    return jax.nn.gelu(x, approximate=True)
def _silu(x):
    return jax.nn.silu(x)
def _sigmoid(x):
    return jax.nn.sigmoid(x)
def _layernorm(x, axis=-1, eps=1e-5):
    m = jnp.mean(x, axis=axis, keepdims=True)
    v = jnp.var(x, axis=axis, keepdims=True)
    return (x - m) / jnp.sqrt(v + eps)
def _scatter_add(tgt, idx, src, axis=0):
    return tgt.at[idx].add(src)
def _segment_sum(src, seg, n):
    return jax.ops.segment_sum(src, seg, n)
class _Rng:
    def __init__(self, key):
        self._k = key
    def _next(self):
        self._k, sub = jax.random.split(self._k)
        return sub
    def normal(self, shape):
        return jax.random.normal(self._next(), shape, dtype=jnp.bfloat16)
    def randint(self, lo, hi, shape):
        return jax.random.randint(self._next(), shape, lo, hi, dtype=jnp.int32)
    def uniform(self, shape, lo=0.0, hi=1.0):
        return jax.random.uniform(self._next(), shape, jnp.bfloat16, lo, hi)
    def permutation(self, n):
        return jax.random.permutation(self._next(), n)


kernel_name = 'concat_heads__sliding_block_cached__sliding_block_cached__decode'

def setup_inputs():
    _rng = _Rng(jax.random.key(int.from_bytes(__import__("os").urandom(4), "little")))
    _w = (lambda a: (lambda t: t.astype(jnp.bfloat16) if jnp.issubdtype(t.dtype, jnp.floating) else t)(jnp.asarray(a)))
    def _A_setup():
        B, Sq, D = 2, 1, 640
        Hq, Hkv, Sk, Dh = 32, 32, 4096, 128
        assert Hq % Hkv == 0, (Hq, Hkv)
        return {
            "x": _w((lambda *s: _rng.normal(s) * 0.8)(B, Sq, D)),
            "k_cache": _w((lambda *s: _rng.normal(s) * 0.8)(B, Hkv, Sk, Dh)),
            "v_cache": _w((lambda *s: _rng.normal(s) * 0.05)(B, Hkv, Sk, Dh)),
            "wq": _w((lambda *s: _rng.normal(s) * 0.8)(D, Hq * Dh) * (D ** -0.5)),
            "wo": _w((lambda *s: _rng.normal(s) * 0.05)(Hq * Dh, D) * ((Hq * Dh) ** -0.5)),
        }
    _A_in = _A_setup()

    def _B_setup():
        B, Sq, D = 2, 1, 640
        Hq, Hkv, Sk, Dh = 32, 32, 4096, 128
        assert Hq % Hkv == 0, (Hq, Hkv)
        return {
            "x": _w((lambda *s: _rng.normal(s) * 0.8)(B, Sq, D)),
            "k_cache": _w((lambda *s: _rng.normal(s) * 0.8)(B, Hkv, Sk, Dh)),
            "v_cache": _w((lambda *s: _rng.normal(s) * 0.05)(B, Hkv, Sk, Dh)),
            "wq": _w((lambda *s: _rng.normal(s) * 0.8)(D, Hq * Dh) * (D ** -0.5)),
            "wo": _w((lambda *s: _rng.normal(s) * 0.05)(Hq * Dh, D) * ((Hq * Dh) ** -0.5)),
        }
    _B_in = _B_setup()

    return {
        "A_x": _A_in["x"],
        "A_k_cache": _A_in["k_cache"],
        "A_v_cache": _A_in["v_cache"],
        "A_wq": _A_in["wq"],
        "A_wo": _A_in["wo"],
        "B_x": _B_in["x"],
        "B_k_cache": _B_in["k_cache"],
        "B_v_cache": _B_in["v_cache"],
        "B_wq": _B_in["wq"],
        "B_wo": _B_in["wo"],
    }

def reference(A_x, A_k_cache, A_v_cache, A_wq, A_wo, B_x, B_k_cache, B_v_cache, B_wq, B_wo):
    def _A_ref(x, k_cache, v_cache, wq, wo):
        B, Sq, D = x.shape
        Hq, Dh = 32, 128
        Hkv, Sk = k_cache.shape[1], k_cache.shape[2]
        W = min(4096, max(256, Sk // 4))
        rep = Hq // Hkv
        q = (lambda x, *d: x.transpose(*d))((x @ wq).reshape(B, Sq, Hq, Dh), 0, 2, 1, 3)
        k = jnp.repeat(k_cache[:, :, Sk - W:, :], rep, axis=1)
        v = jnp.repeat(v_cache[:, :, Sk - W:, :], rep, axis=1)
        scores = jnp.einsum("bhqd,bhkd->bhqk", q, k) * (Dh ** -0.5)
        p = _softmax(scores, axis=-1)
        o = jnp.einsum("bhqk,bhkd->bhqd", p, v)
        return (lambda x, *d: x.transpose(*d))(o, 0, 2, 1, 3).reshape(B, Sq, Hq * Dh) @ wo

    def _B_ref(x, k_cache, v_cache, wq, wo):
        B, Sq, D = x.shape
        Hq, Dh = 32, 128
        Hkv, Sk = k_cache.shape[1], k_cache.shape[2]
        W = min(4096, max(256, Sk // 4))
        rep = Hq // Hkv
        q = (lambda x, *d: x.transpose(*d))((x @ wq).reshape(B, Sq, Hq, Dh), 0, 2, 1, 3)
        k = jnp.repeat(k_cache[:, :, Sk - W:, :], rep, axis=1)
        v = jnp.repeat(v_cache[:, :, Sk - W:, :], rep, axis=1)
        scores = jnp.einsum("bhqd,bhkd->bhqk", q, k) * (Dh ** -0.5)
        p = _softmax(scores, axis=-1)
        o = jnp.einsum("bhqk,bhkd->bhqd", p, v)
        return (lambda x, *d: x.transpose(*d))(o, 0, 2, 1, 3).reshape(B, Sq, Hq * Dh) @ wo

    a = _A_ref(A_x, A_k_cache, A_v_cache, A_wq, A_wo)
    b = _B_ref(B_x, B_k_cache, B_v_cache, B_wq, B_wo)
    return jnp.concatenate([a, b], axis=-1)
```

```python
import functools
import jax
import jax.numpy as jnp
from jax import lax
import jax.experimental.pallas as pl
import jax.experimental.pallas.tpu as pltpu

NP = 2
RING = 3
WO_SCHED = ((1024, 1024, 1024, 1024), (1024, 1024, 1024, 512, 256, 128, 64, 32, 32))
SCOPES = False


def _scope(name):
    import contextlib
    return jax.named_scope(name) if SCOPES else contextlib.nullcontext()


def _kernel(xa, ka, va, wqa, woa, xb, kb, vb, wqb, wob, o_ref,
            x_buf, wq_buf, k_buf, v_buf, wo_buf, o_buf, sem,
            *, nb, nh, sk, w, dh, d):
    probs = ((xa, ka, va, wqa, woa), (xb, kb, vb, wqb, wob))
    scale = dh ** -0.5

    def x_copies():
        return [pltpu.make_async_copy(probs[p][0], x_buf.at[p], sem.at[RING - 1]) for p in range(NP)]

    def head_copies(h, slot):
        cs = []
        for p in range(NP):
            _, k, v, wq, _ = probs[p]
            col = h * dh if isinstance(h, int) else pl.multiple_of(h * dh, dh)
            cs.append(pltpu.make_async_copy(wq.at[:, pl.ds(col, dh)], wq_buf.at[slot, p], sem.at[slot]))
            cs.append(pltpu.make_async_copy(k.at[:, h, pl.ds(sk - w, w), :], k_buf.at[slot, p], sem.at[slot]))
            cs.append(pltpu.make_async_copy(v.at[:, h, pl.ds(sk - w, w), :], v_buf.at[slot, p], sem.at[slot]))
        return cs

    wo_chunks = []
    for p in range(NP):
        r0 = 0
        for r in WO_SCHED[p]:
            wo_chunks.append((p, r0, r))
            r0 += r
        assert r0 == nh * dh

    def wo_copy(c):
        p, r0, r = wo_chunks[c]
        return pltpu.make_async_copy(probs[p][4].at[pl.ds(r0, r), :], wo_buf.at[p, pl.ds(r0, r), :],
                                     sem.at[(nh + c) % RING])

    nslot = RING + 1

    def head_copies2(h):
        cs = []
        s_sem = h % RING
        s_buf = h % nslot
        for p in range(NP):
            _, k, v, wq, _ = probs[p]
            col = h * dh if isinstance(h, int) else pl.multiple_of(h * dh, dh)
            cs.append(pltpu.make_async_copy(wq.at[:, pl.ds(col, dh)], wq_buf.at[s_buf, p], sem.at[s_sem]))
            cs.append(pltpu.make_async_copy(k.at[:, h, pl.ds(sk - w, w), :], k_buf.at[s_buf, p], sem.at[s_sem]))
            cs.append(pltpu.make_async_copy(v.at[:, h, pl.ds(sk - w, w), :], v_buf.at[s_buf, p], sem.at[s_sem]))
        return cs

    with _scope('prologue'):
        for c in head_copies2(0):
            c.start()
        for c in x_copies():
            c.start()
        for g in range(1, RING - 1):
            for c in head_copies2(g):
                c.start()
        for c in x_copies():
            c.wait()
        for c in head_copies2(RING - 1):
            c.start()

    def attn_step(h, n_wo_issue):
        for c in head_copies2(h):
            c.wait()
        if n_wo_issue is None:
            for c in head_copies2(h + RING):
                c.start()
        else:
            wo_copy(n_wo_issue).start()
        s = h % nslot
        for p in range(NP):
            q = jnp.dot(x_buf[p], wq_buf[s, p], preferred_element_type=jnp.float32) * scale
            q = q.astype(jnp.bfloat16)
            rows = []
            for b in range(nb):
                sc = lax.dot_general(q[b:b + 1], k_buf[s, p, b], (((1,), (1,)), ((), ())),
                                     preferred_element_type=jnp.float32)
                m = jnp.max(sc, axis=-1, keepdims=True)
                e = jnp.exp(sc - m)
                l = jnp.sum(e, axis=-1, keepdims=True)
                o = jnp.dot(e.astype(jnp.bfloat16), v_buf[s, p, b], preferred_element_type=jnp.float32)
                rows.append(o / l)
            o_buf[p, h] = jnp.concatenate(rows, axis=0).astype(jnp.bfloat16)

    with _scope('attn'):
        def body(h, carry):
            attn_step(h, None)
            return carry
        lax.fori_loop(0, nh - RING, body, 0)
        for i in range(RING):
            attn_step(nh - RING + i, i)

    with _scope('oproj'):
        acc = None
        for c, (p, r0, r) in enumerate(wo_chunks):
            if r >= dh:
                o = jnp.concatenate([o_buf[p, r0 // dh + i] for i in range(r // dh)], axis=1) if r > dh else o_buf[p, r0 // dh]
            else:
                o = o_buf[p, r0 // dh][:, r0 % dh:r0 % dh + r]
            wo_copy(c).wait()
            if c + RING < len(wo_chunks):
                wo_copy(c + RING).start()
            part = jnp.dot(o, wo_buf[p, r0:r0 + r, :], preferred_element_type=jnp.float32)
            acc = part if r0 == 0 else acc + part
            if r0 + r == nh * dh:
                o_ref[:, p * d:(p + 1) * d] = acc.astype(o_ref.dtype)


@jax.jit
def pallas_concat_heads__sliding_block_cached__sliding_block_cached__decode_kernel(
    A_x, A_k_cache, A_v_cache, A_wq, A_wo, B_x, B_k_cache, B_v_cache, B_wq, B_wo,
):
    B, Sq, D = A_x.shape
    _, H, Sk, Dh = A_k_cache.shape
    W = min(4096, max(256, Sk // 4))
    assert Sq == 1
    dt = A_x.dtype
    ns = RING + 1

    anyspec = pl.BlockSpec(memory_space=pl.ANY)
    out = pl.pallas_call(
        functools.partial(_kernel, nb=B, nh=H, sk=Sk, w=W, dh=Dh, d=D),
        in_specs=[anyspec] * 10,
        out_specs=pl.BlockSpec(memory_space=pltpu.VMEM),
        out_shape=jax.ShapeDtypeStruct((B, NP * D), dt),
        scratch_shapes=[
            pltpu.VMEM((NP, B, D), dt),
            pltpu.VMEM((ns, NP, D, Dh), dt),
            pltpu.VMEM((ns, NP, B, W, Dh), dt),
            pltpu.VMEM((ns, NP, B, W, Dh), dt),
            pltpu.VMEM((NP, H * Dh, D), dt),
            pltpu.VMEM((NP, H, B, Dh), dt),
            pltpu.SemaphoreType.DMA((RING,)),
        ],
        compiler_params=pltpu.CompilerParams(vmem_limit_bytes=64 * 1024 * 1024),
    )(A_x.reshape(B, D), A_k_cache, A_v_cache, A_wq, A_wo,
      B_x.reshape(B, D), B_k_cache, B_v_cache, B_wq, B_wo)
    return out.reshape(B, Sq, NP * D)
```

```python
import functools

import jax
import jax.numpy as jnp
from jax import lax
import jax.experimental.pallas as pl
import jax.experimental.pallas.tpu as pltpu

NP = 2
RING = 3
HG = 2
WO_SCHED = ((8, 8, 8, 8), (8, 8, 8, 4, 3, 1))


def _kernel(xa, ka, va, wqa, woa, xb, kb, vb, wqb, wob, o_ref,
            x_buf, wq_buf, k_buf, v_buf, wo_buf, o_buf, sem,
            *, nb, nh, sk, w, dh, d):
    probs = ((xa, ka, va, wqa, woa), (xb, kb, vb, wqb, wob))
    scale = dh ** -0.5
    ng = nh // HG
    nslot = RING + 1
    gw = HG * dh

    def x_copies():
        return [pltpu.make_async_copy(probs[p][0], x_buf.at[p], sem.at[RING - 1])
                for p in range(NP)]

    def group_copies(g):
        s_sem = g % RING
        s_buf = g % nslot
        col = g * gw if isinstance(g, int) else pl.multiple_of(g * gw, gw)
        cs = []
        for p in range(NP):
            _, k, v, wq, _ = probs[p]
            cs.append(pltpu.make_async_copy(
                wq.at[:, pl.ds(col, gw)], wq_buf.at[s_buf, p], sem.at[s_sem]))
            cs.append(pltpu.make_async_copy(
                k.at[:, pl.ds(g * HG, HG), pl.ds(sk - w, w), :], k_buf.at[s_buf, p], sem.at[s_sem]))
            cs.append(pltpu.make_async_copy(
                v.at[:, pl.ds(g * HG, HG), pl.ds(sk - w, w), :], v_buf.at[s_buf, p], sem.at[s_sem]))
        return cs

    wo_chunks = []
    for p in range(NP):
        h0 = 0
        for u in WO_SCHED[p]:
            n = u * nh // 32
            wo_chunks.append((p, h0, n))
            h0 += n
        assert h0 == nh

    def wo_copy(c):
        p, h0, n = wo_chunks[c]
        rows = pl.ds(h0 * dh, n * dh)
        return pltpu.make_async_copy(probs[p][4].at[rows, :], wo_buf.at[p, rows, :],
                                     sem.at[(ng + c) % RING])

    for c in group_copies(0):
        c.start()
    for c in x_copies():
        c.start()
    for g in range(1, RING - 1):
        for c in group_copies(g):
            c.start()
    for c in x_copies():
        c.wait()
    for c in group_copies(RING - 1):
        c.start()

    def attn_step(g, wo_to_issue):
        for c in group_copies(g):
            c.wait()
        if wo_to_issue is None:
            for c in group_copies(g + RING):
                c.start()
        else:
            wo_copy(wo_to_issue).start()
        s = g % nslot
        for p in range(NP):
            q = jnp.dot(x_buf[p], wq_buf[s, p], preferred_element_type=jnp.float32) * scale
            q = q.astype(k_buf.dtype)
            for hh in range(HG):
                rows = []
                for b in range(nb):
                    sc = lax.dot_general(
                        q[b:b + 1, hh * dh:(hh + 1) * dh], k_buf[s, p, b, hh],
                        (((1,), (1,)), ((), ())),
                        preferred_element_type=jnp.float32)
                    m = jnp.max(sc, axis=-1, keepdims=True)
                    e = jnp.exp(sc - m)
                    l = jnp.sum(e, axis=-1, keepdims=True)
                    o = jnp.dot(e.astype(v_buf.dtype), v_buf[s, p, b, hh],
                                preferred_element_type=jnp.float32)
                    rows.append(o / l)
                o_buf[p, g * HG + hh] = jnp.concatenate(rows, axis=0).astype(o_buf.dtype)

    def body(g, carry):
        attn_step(g, None)
        return carry

    lax.fori_loop(0, ng - RING, body, 0)
    for i in range(RING):
        attn_step(ng - RING + i, i)

    acc = None
    for c, (p, h0, n) in enumerate(wo_chunks):
        o = o_buf[p, h0] if n == 1 else jnp.concatenate(
            [o_buf[p, h0 + i] for i in range(n)], axis=1)
        wo_copy(c).wait()
        if c + RING < len(wo_chunks):
            wo_copy(c + RING).start()
        part = jnp.dot(o, wo_buf[p, h0 * dh:(h0 + n) * dh, :],
                       preferred_element_type=jnp.float32)
        acc = part if h0 == 0 else acc + part
        if h0 + n == nh:
            o_ref[:, p * d:(p + 1) * d] = acc.astype(o_ref.dtype)


@jax.jit
def pallas_concat_heads__sliding_block_cached__sliding_block_cached__decode_kernel(
    A_x: jax.Array,
    A_k_cache: jax.Array,
    A_v_cache: jax.Array,
    A_wq: jax.Array,
    A_wo: jax.Array,
    B_x: jax.Array,
    B_k_cache: jax.Array,
    B_v_cache: jax.Array,
    B_wq: jax.Array,
    B_wo: jax.Array,
):
    B, Sq, D = A_x.shape
    _, H, Sk, Dh = A_k_cache.shape
    W = min(4096, max(256, Sk // 4))
    assert Sq == 1 and H % 32 == 0 and H // HG > RING
    assert A_wq.shape == (D, H * Dh) and A_wo.shape == (H * Dh, D)
    dt = A_x.dtype
    ns = RING + 1

    hbm = pl.BlockSpec(memory_space=pl.ANY)
    out = pl.pallas_call(
        functools.partial(_kernel, nb=B, nh=H, sk=Sk, w=W, dh=Dh, d=D),
        in_specs=[hbm] * 10,
        out_specs=pl.BlockSpec(memory_space=pltpu.VMEM),
        out_shape=jax.ShapeDtypeStruct((B, NP * D), dt),
        scratch_shapes=[
            pltpu.VMEM((NP, B, D), dt),
            pltpu.VMEM((ns, NP, D, HG * Dh), dt),
            pltpu.VMEM((ns, NP, B, HG, W, Dh), dt),
            pltpu.VMEM((ns, NP, B, HG, W, Dh), dt),
            pltpu.VMEM((NP, H * Dh, D), dt),
            pltpu.VMEM((NP, H, B, Dh), dt),
            pltpu.SemaphoreType.DMA((RING,)),
        ],
        compiler_params=pltpu.CompilerParams(vmem_limit_bytes=64 * 1024 * 1024),
    )(A_x.reshape(B, D), A_k_cache, A_v_cache, A_wq, A_wo,
      B_x.reshape(B, D), B_k_cache, B_v_cache, B_wq, B_wo)
    return out.reshape(B, Sq, NP * D)
```

```python
import functools

import jax
import jax.numpy as jnp
from jax import lax
import jax.experimental.pallas as pl
import jax.experimental.pallas.tpu as pltpu

NP = 2
RING = 3
HG = 2
LANES = 128
WO_SCHED = ((8, 8, 8, 8), (8, 8, 8, 4, 2))
VPU_PIECES = (160, 64, 32)


def _kernel(xa, ka, va, wqa, woa, xb, kb, vb, wqb, wob, o_ref,
            x_buf, wq_buf, k_buf, v_buf, wo_buf, o_buf, ocb_buf, sem,
            *, nb, nh, sk, w, dh, d):
    probs = ((xa, ka, va, wqa, woa), (xb, kb, vb, wqb, wob))
    scale = dh ** -0.5
    ng = nh // HG
    nslot = RING + 1
    gw = HG * dh

    def x_copies():
        return [pltpu.make_async_copy(probs[p][0], x_buf.at[p], sem.at[RING - 1])
                for p in range(NP)]

    def group_copies(g):
        s_sem = g % RING
        s_buf = g % nslot
        col = g * gw if isinstance(g, int) else pl.multiple_of(g * gw, gw)
        cs = []
        for p in range(NP):
            _, k, v, wq, _ = probs[p]
            cs.append(pltpu.make_async_copy(
                wq.at[:, pl.ds(col, gw)], wq_buf.at[s_buf, p], sem.at[s_sem]))
            cs.append(pltpu.make_async_copy(
                k.at[:, pl.ds(g * HG, HG), pl.ds(sk - w, w), :], k_buf.at[s_buf, p], sem.at[s_sem]))
            cs.append(pltpu.make_async_copy(
                v.at[:, pl.ds(g * HG, HG), pl.ds(sk - w, w), :], v_buf.at[s_buf, p], sem.at[s_sem]))
        return cs

    wo_chunks = []
    vpu_r0 = nh * dh - sum(VPU_PIECES)
    for p in range(NP):
        r0 = 0
        for u in WO_SCHED[p]:
            n = u * nh // 32 * dh
            wo_chunks.append((p, r0, n, False))
            r0 += n
        if p == NP - 1:
            assert r0 == vpu_r0
            for n in VPU_PIECES:
                wo_chunks.append((p, r0, n, True))
                r0 += n
        assert r0 == nh * dh

    def wo_copy(c):
        p, r0, n, _ = wo_chunks[c]
        rows = pl.ds(r0, n)
        return pltpu.make_async_copy(probs[p][4].at[rows, :], wo_buf.at[p, rows, :],
                                     sem.at[(ng + c) % RING])

    for c in group_copies(0):
        c.start()
    for c in x_copies():
        c.start()
    for g in range(1, RING - 1):
        for c in group_copies(g):
            c.start()
    for c in x_copies():
        c.wait()
    for c in group_copies(RING - 1):
        c.start()

    def attn_step(g, wo_to_issue):
        for c in group_copies(g):
            c.wait()
        if wo_to_issue is None:
            for c in group_copies(g + RING):
                c.start()
        else:
            wo_copy(wo_to_issue).start()
        s = g % nslot
        for p in range(NP):
            q = jnp.dot(x_buf[p], wq_buf[s, p], preferred_element_type=jnp.float32)
            q = q.astype(k_buf.dtype)
            for hh in range(HG):
                rows = []
                for b in range(nb):
                    sc = lax.dot_general(
                        q[b:b + 1, hh * dh:(hh + 1) * dh], k_buf[s, p, b, hh],
                        (((1,), (1,)), ((), ())),
                        preferred_element_type=jnp.float32) * scale
                    m = jnp.max(sc, axis=-1, keepdims=True)
                    e = jnp.exp(sc - m)
                    l = jnp.sum(e, axis=-1, keepdims=True)
                    o = jnp.dot(e.astype(v_buf.dtype), v_buf[s, p, b, hh],
                                preferred_element_type=jnp.float32)
                    rows.append(o / l)
                o_buf[p, g * HG + hh] = jnp.concatenate(rows, axis=0).astype(o_buf.dtype)

    def body(g, carry):
        attn_step(g, None)
        return carry

    lax.fori_loop(0, ng - RING, body, 0)
    for i in range(RING):
        attn_step(ng - RING + i, i)

    acc = None
    accv = None
    for c, (p, r0, n, on_vpu) in enumerate(wo_chunks):
        if not on_vpu:
            h0 = r0 // dh
            o = jnp.concatenate([o_buf[p, h0 + i] for i in range(n // dh)], axis=1)
        wo_copy(c).wait()
        if c + RING < len(wo_chunks):
            wo_copy(c + RING).start()
        if not on_vpu:
            part = jnp.dot(o, wo_buf[p, r0:r0 + n, :], preferred_element_type=jnp.float32)
            acc = part if r0 == 0 else acc + part
            if c == 0:
                eye = (lax.broadcasted_iota(jnp.int32, (dh, dh), 0)
                       == lax.broadcasted_iota(jnp.int32, (dh, dh), 1))
                for h in range(vpu_r0 // dh, nh):
                    of = o_buf[NP - 1, h].astype(jnp.float32)
                    for b in range(nb):
                        col = jnp.sum(jnp.where(eye, of[b:b + 1], 0.0), axis=1, keepdims=True)
                        ocb_buf[b, h * dh - vpu_r0:(h + 1) * dh - vpu_r0, :] = (
                            jnp.broadcast_to(col, (dh, LANES)))
        else:
            parts = []
            for b in range(nb):
                ocb = ocb_buf[b, r0 - vpu_r0:r0 - vpu_r0 + n, :]
                tiles = []
                for j in range(d // LANES):
                    wf = wo_buf[p, r0:r0 + n, j * LANES:(j + 1) * LANES].astype(jnp.float32)
                    tiles.append(jnp.sum((wf * ocb).reshape(n // 8, 8, LANES), axis=0))
                parts.append(jnp.concatenate(tiles, axis=1))
            accv = parts if accv is None else [a + t for a, t in zip(accv, parts)]
        if r0 + n == nh * dh:
            if on_vpu:
                acc = acc + jnp.concatenate(
                    [jnp.sum(a, axis=0, keepdims=True) for a in accv], axis=0)
            o_ref[:, p * d:(p + 1) * d] = acc.astype(o_ref.dtype)


@jax.jit
def pallas_concat_heads__sliding_block_cached__sliding_block_cached__decode_kernel(
    A_x: jax.Array,
    A_k_cache: jax.Array,
    A_v_cache: jax.Array,
    A_wq: jax.Array,
    A_wo: jax.Array,
    B_x: jax.Array,
    B_k_cache: jax.Array,
    B_v_cache: jax.Array,
    B_wq: jax.Array,
    B_wo: jax.Array,
):
    B, Sq, D = A_x.shape
    _, H, Sk, Dh = A_k_cache.shape
    W = min(4096, max(256, Sk // 4))
    assert Sq == 1 and H % 32 == 0 and H // HG > RING and D % LANES == 0
    assert A_wq.shape == (D, H * Dh) and A_wo.shape == (H * Dh, D)
    assert sum(VPU_PIECES) % Dh == 0 and all(n % 16 == 0 for n in VPU_PIECES)
    dt = A_x.dtype
    ns = RING + 1

    hbm = pl.BlockSpec(memory_space=pl.ANY)
    out = pl.pallas_call(
        functools.partial(_kernel, nb=B, nh=H, sk=Sk, w=W, dh=Dh, d=D),
        in_specs=[hbm] * 10,
        out_specs=pl.BlockSpec(memory_space=pltpu.VMEM),
        out_shape=jax.ShapeDtypeStruct((B, NP * D), dt),
        scratch_shapes=[
            pltpu.VMEM((NP, B, D), dt),
            pltpu.VMEM((ns, NP, D, HG * Dh), dt),
            pltpu.VMEM((ns, NP, B, HG, W, Dh), dt),
            pltpu.VMEM((ns, NP, B, HG, W, Dh), dt),
            pltpu.VMEM((NP, H * Dh, D), dt),
            pltpu.VMEM((NP, H, B, Dh), dt),
            pltpu.VMEM((B, sum(VPU_PIECES), LANES), jnp.float32),
            pltpu.SemaphoreType.DMA((RING,)),
        ],
        compiler_params=pltpu.CompilerParams(vmem_limit_bytes=64 * 1024 * 1024),
    )(A_x.reshape(B, D), A_k_cache, A_v_cache, A_wq, A_wo,
      B_x.reshape(B, D), B_k_cache, B_v_cache, B_wq, B_wo)
    return out.reshape(B, Sq, NP * D)
```
